```python
import jax
import jax.numpy as jnp

def _softmax(x, axis=-1):
    return jax.nn.softmax(x, axis=axis)
def _gelu(x):
    return jax.nn.gelu(x, approximate=True)
def _silu(x):
    return jax.nn.silu(x)
def _sigmoid(x):
    return jax.nn.sigmoid(x)
def _layernorm(x, axis=-1, eps=1e-5):
    m = jnp.mean(x, axis=axis, keepdims=True)
    v = jnp.var(x, axis=axis, keepdims=True)
    return (x - m) / jnp.sqrt(v + eps)
def _scatter_add(tgt, idx, src, axis=0):
    return tgt.at[idx].add(src)
def _segment_sum(src, seg, n):
    return jax.ops.segment_sum(src, seg, n)
class _Rng:
    def __init__(self, key):
        self._k = key
    def _next(self):
        self._k, sub = jax.random.split(self._k)
        return sub
    def normal(self, shape):
        return jax.random.normal(self._next(), shape, dtype=jnp.bfloat16)
    def randint(self, lo, hi, shape):
        return jax.random.randint(self._next(), shape, lo, hi, dtype=jnp.int32)
    def uniform(self, shape, lo=0.0, hi=1.0):
        return jax.random.uniform(self._next(), shape, jnp.bfloat16, lo, hi)
    def permutation(self, n):
        return jax.random.permutation(self._next(), n)


kernel_name = 'concat_heads__compressed_kv_cla__gqa_block_cached__decode'

def setup_inputs():
    _rng = _Rng(jax.random.key(int.from_bytes(__import__("os").urandom(4), "little")))
    _w = (lambda a: (lambda t: t.astype(jnp.bfloat16) if jnp.issubdtype(t.dtype, jnp.floating) else t)(jnp.asarray(a)))
    def _A_setup():
        B, H, Sq, Sk, D, M = 2, 32, 1, 4096, 128, 512
        Dc = 4 * D
        return {
            "x": _w((lambda *s: _rng.normal(s) * 0.05)(B, Sq, M)),
            "c_kv": _w((lambda *s: _rng.normal(s) * 0.05)(B, Sk, Dc)),
            "w_q": _w((lambda *s: _rng.normal(s) * 0.05)(M, H, D) * (M ** -0.5)),
            "w_uk": _w((lambda *s: _rng.normal(s) * 0.05)(Dc, H, D) * (Dc ** -0.5)),
            "w_uv": _w((lambda *s: _rng.normal(s) * 0.05)(Dc, H, D) * (Dc ** -0.5)),
            "w_o": _w((lambda *s: _rng.normal(s) * 0.05)(H, D, M) * ((H * D) ** -0.5)),
        }
    _A_in = _A_setup()

    def _B_setup():
        B, Sq, D = 2, 1, 512
        Hq, Hkv, Sk, Dh = 32, 32, 4096, 128
        assert Hq % Hkv == 0, (Hq, Hkv)
        return {
            "x": _w((lambda *s: _rng.normal(s) * 0.05)(B, Sq, D)),
            "k_cache": _w((lambda *s: _rng.normal(s) * 0.05)(B, Hkv, Sk, Dh)),
            "v_cache": _w((lambda *s: _rng.normal(s) * 0.05)(B, Hkv, Sk, Dh)),
            "wq": _w((lambda *s: _rng.normal(s) * 0.05)(D, Hq * Dh) * (D ** -0.5)),
            "wo": _w((lambda *s: _rng.normal(s) * 0.05)(Hq * Dh, D) * ((Hq * Dh) ** -0.5)),
        }
    _B_in = _B_setup()

    return {
        "A_x": _A_in["x"],
        "A_c_kv": _A_in["c_kv"],
        "A_w_q": _A_in["w_q"],
        "A_w_uk": _A_in["w_uk"],
        "A_w_uv": _A_in["w_uv"],
        "A_w_o": _A_in["w_o"],
        "B_x": _B_in["x"],
        "B_k_cache": _B_in["k_cache"],
        "B_v_cache": _B_in["v_cache"],
        "B_wq": _B_in["wq"],
        "B_wo": _B_in["wo"],
    }

def reference(A_x, A_c_kv, A_w_q, A_w_uk, A_w_uv, A_w_o, B_x, B_k_cache, B_v_cache, B_wq, B_wo):
    def _A_ref(x, c_kv, w_q, w_uk, w_uv, w_o):
        B, Sq, M = x.shape[0], x.shape[1], x.shape[2]
        Sk = c_kv.shape[1]
        H, D = w_q.shape[1], w_q.shape[2]
        q = jnp.einsum("bqm,mhd->bhqd", x, w_q)
        k = jnp.einsum("bkc,chd->bhkd", c_kv, w_uk)
        v = jnp.einsum("bkc,chd->bhkd", c_kv, w_uv)
        scores = jnp.einsum("bhqd,bhkd->bhqk", q, k) * (D ** -0.5)
        off = Sk - Sq
        qi = jnp.arange(Sq)[:, None]
        kj = jnp.arange(Sk)[None, :]
        cmask = kj <= (qi + off)
        scores = jnp.where(cmask[None, None], scores, -1e9)
        p = _softmax(scores, axis=-1)
        ctx = jnp.einsum("bhqk,bhkd->bhqd", p, v)
        return jnp.einsum("bhqd,hdm->bqm", ctx, w_o)

    def _B_ref(x, k_cache, v_cache, wq, wo):
        B, Sq, D = x.shape
        Hq, Dh = 32, 128
        Hkv = k_cache.shape[1]
        rep = Hq // Hkv
        q = (lambda x, *d: x.transpose(*d))((x @ wq).reshape(B, Sq, Hq, Dh), 0, 2, 1, 3)
        k = jnp.repeat(k_cache, rep, axis=1)
        v = jnp.repeat(v_cache, rep, axis=1)
        scores = jnp.einsum("bhqd,bhkd->bhqk", q, k) * (Dh ** -0.5)
        p = _softmax(scores, axis=-1)
        o = jnp.einsum("bhqk,bhkd->bhqd", p, v)
        return (lambda x, *d: x.transpose(*d))(o, 0, 2, 1, 3).reshape(B, Sq, Hq * Dh) @ wo

    a = _A_ref(A_x, A_c_kv, A_w_q, A_w_uk, A_w_uv, A_w_o)
    b = _B_ref(B_x, B_k_cache, B_v_cache, B_wq, B_wo)
    return jnp.concatenate([a, b], axis=-1)
```

```python
import jax
import jax.numpy as jnp
from jax import lax
import jax.experimental.pallas as pl
import jax.experimental.pallas.tpu as pltpu

_BF16 = jnp.bfloat16
_F32 = jnp.float32

_B = 2
_H = 32
_D = 128
_M = 512
_S = 4096

_G = 4
_NSLOT = 3
_UNITS = 16
_LAG = 4

_ROWS128 = ((0, 80), (80, 96), (176, 80))
_ROWS512 = ((0, 24), (24, 24), (48, 16))
_COLS4096 = ((0, 1536), (1536, 1280), (2816, 1280))


def _aligned(x, m):
    return x if isinstance(x, int) else pl.multiple_of(x, m)


def _start_unit(streams):
    for c in range(3):
        for i, stream in enumerate(streams):
            src, dst, sem = stream[c]
            pltpu.make_async_copy(src, dst, sem).start(priority=i % 2)


def _wait_whole(buf, sem):
    pltpu.make_async_copy(buf, buf, sem).wait()


def _nt_dot(a, b):
    return lax.dot_general(a, b, (((1,), (1,)), ((), ())), preferred_element_type=_F32)


def _dot(a, b):
    return jnp.dot(a, b, preferred_element_type=_F32)


def _loop(n, body, init=None):
    return lax.fori_loop(0, n, body, init)


def _kernel(
    ax_hbm, ckv_hbm, awq_hbm, awuk_hbm, awuv_hbm, awo_hbm,
    bx_hbm, k_hbm, v_hbm, bwq_hbm, bwo_hbm,
    out_ref,
    ax_v, bx_v, bwq_v, awq_v, awuk_v, awuv_v, ckv_v, wo_v, kv_v,
    expand_s, xa_s, xb_s, qb_s, ob_s, qa_s, cc_s, ctx_s,
    sem_x, sem_w, sem_kv, sem_o,
):
    def rows(src, dst, sem, base, chunks):
        return [
            (src.at[pl.ds(base + r, n)], dst.at[pl.ds(base + r, n)], sem) for r, n in chunks
        ]

    def q_weights_unit(u):
        streams = []
        for q in range(4):
            r8 = pl.ds(_aligned(q * 128 + u * 8, 8), 8)
            streams.append([
                (bwq_hbm.at[r8, pl.ds(c, n)], bwq_v.at[r8, pl.ds(c, n)], sem_w.at[0])
                for c, n in _COLS4096
            ])
            base = _aligned(q * 4096 + u * 256, 256)
            streams.append(rows(awq_hbm, awq_v, sem_w.at[1], base, _ROWS128))
        _start_unit(streams)

    def up_weights_unit(u):
        streams = []
        for q in range(4):
            base = _aligned(q * 4096 + u * 256, 256)
            streams.append(rows(awuk_hbm, awuk_v, sem_w.at[2], base, _ROWS128))
            streams.append(rows(awuv_hbm, awuv_v, sem_w.at[3], base, _ROWS128))
        _start_unit(streams)

    def latent_unit(u):
        _start_unit([
            rows(ckv_hbm, ckv_v, sem_w.at[4], _aligned(q * 1024 + u * 64, 64), _ROWS512)
            for q in range(8)
        ])

    def kv_unit(u):
        group = u // _UNITS
        slot = group % _NSLOT
        base = _aligned((u % _UNITS) * 256, 256)
        _start_unit([
            [
                (
                    src.at[group * _G + i, pl.ds(base + r, n)],
                    kv_v.at[slot, which, i, pl.ds(base + r, n)],
                    sem_kv.at[slot],
                )
                for r, n in _ROWS128
            ]
            for i in range(_G)
            for which, src in enumerate((k_hbm, v_hbm))
        ])

    def out_weights_unit(u):
        piece = u // 2
        base = _aligned((u % 2) * 64, 64)
        _start_unit([
            [
                (
                    src.at[pl.ds(_aligned(q * 1024 + u * 64, 64) + r, n)],
                    wo_v.at[piece, which, q, pl.ds(base + r, n)],
                    sem_o.at[piece],
                )
                for r, n in _ROWS512
            ]
            for q in range(4)
            for which, src in enumerate((awo_hbm, bwo_hbm))
        ])

    def issue(unit_fn, first, count):
        def body(i, _):
            unit_fn(first + i)

        _loop(count, body)

    def issue_across(j, per_step, unit_fn, next_fn):
        own_steps = (_UNITS - _LAG) // per_step
        pl.when(j < own_steps)(lambda: issue(unit_fn, _LAG + j * per_step, per_step))
        pl.when(j >= own_steps)(lambda: issue(next_fn, (j - own_steps) * per_step, per_step))

    x_copies = [
        pltpu.make_async_copy(ax_hbm, ax_v, sem_x.at[0]),
        pltpu.make_async_copy(bx_hbm, bx_v, sem_x.at[1]),
    ]
    q_weights_unit(0)
    for c in x_copies:
        c.start()
    issue(q_weights_unit, 1, _UNITS - 1)
    issue(up_weights_unit, 0, _LAG)

    def build_expand(i, _):
        r0 = pl.multiple_of(i * 16, 16)
        row = lax.broadcasted_iota(jnp.int32, (16, 128 * _H), 0) + r0
        col = lax.broadcasted_iota(jnp.int32, (16, 128 * _H), 1)
        expand_s[pl.ds(r0, 16), :] = jnp.where(col // _H == row, 1.0, 0.0).astype(_BF16)

    _loop(128 // 16, build_expand)

    def keep_own_head(x):
        row = lax.broadcasted_iota(jnp.int32, (_B * _H, 128), 0)
        col = lax.broadcasted_iota(jnp.int32, (_B * _H, 128), 1)
        own = row % _H == col % _H
        tiles = [
            jnp.where(own, x[:, t : t + 128], 0.0).astype(_BF16)
            for t in range(0, x.shape[1], 128)
        ]
        return jnp.concatenate(tiles, axis=1)

    def per_head_proj(x, w_ref, j):
        lhs = keep_own_head(_dot(x, expand_s[...]))
        return _dot(lhs, w_ref[pl.ds(pl.multiple_of(j * 4096, 4096), 4096), :])

    for c in x_copies:
        c.wait()
    xa = ax_v[...].astype(_F32)
    xb = bx_v[...].astype(_F32)
    sub = lax.broadcasted_iota(jnp.int32, (8, _D), 0)
    for j in range(4):
        cols = slice(j * 128, (j + 1) * 128)
        for b in range(_B):
            xa_s[j, pl.ds(b * _H, _H), :] = jnp.broadcast_to(xa[b : b + 1, cols], (_H, 128))
        xb_s[j] = jnp.where(
            sub == 0,
            jnp.broadcast_to(xb[0:1, cols], (8, 128)),
            jnp.broadcast_to(xb[1:2, cols], (8, 128)),
        )

    _wait_whole(bwq_v, sem_w.at[0])
    _wait_whole(awq_v, sem_w.at[1])

    def q_step(j, carry):
        qa, qb = carry
        w = bwq_v[pl.ds(pl.multiple_of(j * 128, 128), 128), :]
        qb = qb + _dot(xb_s[j].astype(_BF16), w)
        qa = qa + per_head_proj(xa_s[j].astype(_BF16), awq_v, j)
        issue_across(j, 4, up_weights_unit, latent_unit)
        return qa, qb

    qa, qb = _loop(
        4, q_step, (jnp.zeros((_B * _H, _D), _F32), jnp.zeros((8, _H * _D), _F32))
    )
    for h in range(_H):
        for b in range(_B):
            qb_s[pl.ds(b * _H + h, 1), :] = qb[b : b + 1, h * _D : (h + 1) * _D]
    qa = qa.astype(_BF16)

    _wait_whole(awuk_v, sem_w.at[2])
    _wait_whole(awuv_v, sem_w.at[3])

    def absorb_step(j, _):
        w = awuk_v[pl.ds(pl.multiple_of(j * 4096, 4096), 4096), :]
        qa_s[j] = _nt_dot(keep_own_head(_nt_dot(qa, w)), expand_s[...])
        issue_across(j, 4, latent_unit, kv_unit)

    _loop(4, absorb_step)

    _wait_whole(ckv_v, sem_w.at[4])
    scale = _D ** -0.5
    kv_issued = _LAG

    def latent_batch(b, _):
        heads = pl.ds(pl.multiple_of(b * _H, _H), _H)
        q = jnp.concatenate([qa_s[j, heads, :] for j in range(4)], axis=1).astype(_BF16)

        def block(j, carry):
            m, l, acc = carry
            c = ckv_v[pl.ds(pl.multiple_of(b * _S + j * 1024, 1024), 1024), :]
            s = _nt_dot(q, c)
            m_new = jnp.maximum(m, jnp.max(s, axis=1, keepdims=True))
            alpha = jnp.exp((m - m_new) * scale)
            p = jnp.exp((s - m_new) * scale)
            l = alpha * l + jnp.sum(p, axis=1, keepdims=True)
            acc = alpha * acc + _dot(p.astype(_BF16), c)
            issue(kv_unit, kv_issued + (b * 4 + j) * 2, 2)
            return m_new, l, acc

        init = (
            jnp.full((_H, 1), -jnp.inf, _F32),
            jnp.zeros((_H, 1), _F32),
            jnp.zeros((_H, _M), _F32),
        )
        _, l, acc = _loop(4, block, init)
        cc = acc / l
        for j in range(4):
            cc_s[j, heads, :] = cc[:, j * 128 : (j + 1) * 128]

    _loop(_B, latent_batch)
    kv_issued += 16

    def value_step(j, ctx):
        ctx = ctx + per_head_proj(cc_s[j].astype(_BF16), awuv_v, j)
        issue(kv_unit, kv_issued + j * 2, 2)
        return ctx

    ctx_s[...] = _loop(4, value_step, jnp.zeros((_B * _H, _D), _F32))
    kv_issued += 8

    n_heads = _B * _H
    kv_steps = (n_heads * 4 - kv_issued) // 4
    assert _UNITS + _LAG <= kv_issued <= (_NSLOT - 1) * _UNITS
    out_issued = 2 * (n_heads - kv_steps)
    assert out_issued <= _UNITS

    def head_step(t, _):
        group, i = t // _G, t % _G
        slot = group % _NSLOT

        def issue_half(half):
            pl.when(t < kv_steps)(lambda: issue(kv_unit, kv_issued + 4 * t + 2 * half, 2))
            pl.when(t >= kv_steps)(lambda: out_weights_unit(2 * (t - kv_steps) + half))

        pl.when(i == 0)(lambda: _wait_whole(kv_v.at[slot], sem_kv.at[slot]))
        q = jnp.broadcast_to(qb_s[pl.ds(t, 1), :], (8, _D)).astype(_BF16)
        s = _nt_dot(q, kv_v[slot, 0, i])
        issue_half(0)
        m = jnp.max(s, axis=1, keepdims=True)
        p = jnp.exp((s - m) * scale)
        l = jnp.sum(p, axis=1, keepdims=True)
        o = _dot(p.astype(_BF16), kv_v[slot, 1, i])
        ob_s[pl.ds(t, 1), :] = (o / l)[0:1]
        issue_half(1)

    _loop(n_heads, head_step)

    def head_rows(ref, h):
        r0 = jnp.broadcast_to(ref[pl.ds(h, 1), :], (8, _D))
        r1 = jnp.broadcast_to(ref[pl.ds(_H + h, 1), :], (8, _D))
        return jnp.where(sub == 0, r0, r1).astype(_BF16)

    def out_step(piece, acc):
        pl.when(out_issued + piece < _UNITS)(lambda: out_weights_unit(out_issued + piece))
        _wait_whole(wo_v.at[piece], sem_o.at[piece])
        acc = list(acc)
        for which, src in enumerate((ctx_s, ob_s)):
            for q in range(4):
                lhs = head_rows(src, q * 8 + piece)
                acc[which] = acc[which] + _dot(lhs, wo_v[piece, which, q])
        return tuple(acc)

    acc = _loop(_UNITS // 2, out_step, (jnp.zeros((8, _M), _F32),) * 2)
    out_ref[...] = jnp.concatenate(acc, axis=1)[0:_B].astype(out_ref.dtype)


@jax.jit
def pallas_concat_heads__compressed_kv_cla__gqa_block_cached__decode_kernel(
    A_x: jax.Array,
    A_c_kv: jax.Array,
    A_w_q: jax.Array,
    A_w_uk: jax.Array,
    A_w_uv: jax.Array,
    A_w_o: jax.Array,
    B_x: jax.Array,
    B_k_cache: jax.Array,
    B_v_cache: jax.Array,
    B_wq: jax.Array,
    B_wo: jax.Array,
):
    assert A_x.shape == B_x.shape == (_B, 1, _M)
    assert A_c_kv.shape == (_B, _S, _M)
    assert A_w_q.shape == A_w_uk.shape == A_w_uv.shape == (_M, _H, _D)
    assert B_k_cache.shape == B_v_cache.shape == (_B, _H, _S, _D)

    hbm = pl.BlockSpec(memory_space=pltpu.HBM)
    dma = pltpu.SemaphoreType.DMA
    out = pl.pallas_call(
        _kernel,
        in_specs=[hbm] * 11,
        out_specs=pl.BlockSpec(memory_space=pltpu.VMEM),
        out_shape=jax.ShapeDtypeStruct((_B, 2 * _M), A_x.dtype),
        scratch_shapes=[
            pltpu.VMEM((_B, _M), _BF16),
            pltpu.VMEM((_B, _M), _BF16),
            pltpu.VMEM((_M, _H * _D), _BF16),
            pltpu.VMEM((_M * _H, _D), _BF16),
            pltpu.VMEM((_M * _H, _D), _BF16),
            pltpu.VMEM((_M * _H, _D), _BF16),
            pltpu.VMEM((_B * _S, _M), _BF16),
            pltpu.VMEM((_UNITS // 2, 2, 4, _D, _M), _BF16),
            pltpu.VMEM((_NSLOT, 2, _G, _S, _D), _BF16),
            pltpu.VMEM((128, 128 * _H), _BF16),
            pltpu.VMEM((4, _B * _H, 128), _F32),
            pltpu.VMEM((4, 8, 128), _F32),
            pltpu.VMEM((_B * _H, _D), _F32),
            pltpu.VMEM((_B * _H, _D), _F32),
            pltpu.VMEM((4, _B * _H, 128), _F32),
            pltpu.VMEM((4, _B * _H, 128), _F32),
            pltpu.VMEM((_B * _H, _D), _F32),
            dma((2,)),
            dma((5,)),
            dma((_NSLOT,)),
            dma((_UNITS // 2,)),
        ],
        compiler_params=pltpu.CompilerParams(vmem_limit_bytes=100 * 2**20, disable_bounds_checks=True),
    )(
        A_x.reshape(_B, _M),
        A_c_kv.reshape(_B * _S, _M),
        A_w_q.reshape(_M * _H, _D),
        A_w_uk.reshape(_M * _H, _D),
        A_w_uv.reshape(_M * _H, _D),
        A_w_o.reshape(_H * _D, _M),
        B_x.reshape(_B, _M),
        B_k_cache.reshape(_B * _H, _S, _D),
        B_v_cache.reshape(_B * _H, _S, _D),
        B_wq,
        B_wo,
    )
    return out.reshape(_B, 1, 2 * _M)
```

```python
import jax
import jax.numpy as jnp
from jax import lax
import jax.experimental.pallas as pl
import jax.experimental.pallas.tpu as pltpu

_BF16 = jnp.bfloat16
_F32 = jnp.float32

_B = 2
_H = 32
_D = 128
_M = 512
_S = 4096

_G = 8
_NSLOT = 3
_UNITS = 8
_LAG = 2


def _chunks(*sizes):
    return tuple((sum(sizes[:i]), n) for i, n in enumerate(sizes))


_ROWS128 = _chunks(64, 64, 192, 64, 128)
_ROWS512 = _chunks(16, 16, 48, 16, 32)
_COLS4096 = _chunks(1024, 1024, 2048, 2048, 2048)


def _aligned(x, m):
    return x if isinstance(x, int) else pl.multiple_of(x, m)


def _start_unit(streams):
    for c in range(len(streams[0])):
        for i, stream in enumerate(streams):
            src, dst, sem = stream[c]
            pltpu.make_async_copy(src, dst, sem).start(priority=i % 2)


def _wait_whole(buf, sem):
    pltpu.make_async_copy(buf, buf, sem).wait()


def _nt_dot(a, b):
    return lax.dot_general(a, b, (((1,), (1,)), ((), ())), preferred_element_type=_F32)


def _dot(a, b):
    return jnp.dot(a, b, preferred_element_type=_F32)


def _loop(n, body, init=None):
    return lax.fori_loop(0, n, body, init)


def _kernel(
    ax_hbm, ckv_hbm, awq_hbm, awuk_hbm, awuv_hbm, awo_hbm,
    bx_hbm, k_hbm, v_hbm, bwq_hbm, bwo_hbm,
    out_ref,
    ax_v, bx_v, bwq_v, awq_v, awuk_v, awuv_v, ckv_v, wo_v, kv_v,
    expand_s, xa_s, xb_s, qb_s, ob_s, qa_s, cc_s, ctx_s,
    sem_x, sem_w, sem_kv, sem_o,
):
    def rows(src, dst, sem, base, chunks):
        return [
            (src.at[pl.ds(base + r, n)], dst.at[pl.ds(base + r, n)], sem) for r, n in chunks
        ]

    def weights_unit(u):
        streams = []
        for q in range(4):
            base = _aligned(q * 128 + u * 16, 16)
            tiles = [
                (pl.ds(base + c // 4096 * 8, 8), pl.ds(c % 4096, n)) for c, n in _COLS4096
            ]
            streams.append([(bwq_hbm.at[t], bwq_v.at[t], sem_w.at[0]) for t in tiles])
            base = _aligned(q * 4096 + u * 512, 512)
            streams.append(rows(awq_hbm, awq_v, sem_w.at[1], base, _ROWS128))
            streams.append(rows(awuk_hbm, awuk_v, sem_w.at[2], base, _ROWS128))
            streams.append(rows(awuv_hbm, awuv_v, sem_w.at[3], base, _ROWS128))
        _start_unit(streams)

    def latent_unit(u):
        _start_unit([
            rows(ckv_hbm, ckv_v, sem_w.at[4], _aligned(q * 1024 + u * 128, 128), _ROWS512)
            for q in range(8)
        ])

    def kv_unit(u, half=None):
        base = _aligned((u % _UNITS) * 512, 512)
        if half in (None, 0):
            kv_chunks(u, base, ((64, 64), (128, 192)))
        if half in (None, 1):
            kv_chunks(u, base, ((320, 64),))
            pl.when(u % _UNITS < _UNITS - 1)(lambda: kv_chunks(u, base, ((384, 192),)))
            pl.when(u % _UNITS == _UNITS - 1)(lambda: kv_chunks(u, 0, ((3968, 128), (0, 64))))

    def kv_chunks(u, base, chunks):
        group = u // _UNITS
        slot = group % _NSLOT
        _start_unit([
            [
                (
                    src.at[group * _G + i, pl.ds(base + r, n)],
                    kv_v.at[slot, which, i, pl.ds(base + r, n)],
                    sem_kv.at[slot],
                )
                for r, n in chunks
            ]
            for i in range(_G)
            for which, src in enumerate((k_hbm, v_hbm))
        ])

    def out_weights_unit(u):
        _start_unit([
            [
                (
                    src.at[pl.ds(_aligned(q * 1024 + u * 128, 128) + r, n)],
                    wo_v.at[u, which, q, pl.ds(r, n)],
                    sem_o.at[u],
                )
                for r, n in _ROWS512
            ]
            for q in range(4)
            for which, src in enumerate((awo_hbm, bwo_hbm))
        ])

    def issue(unit_fn, first, count):
        def body(i, _):
            unit_fn(first + i)

        _loop(count, body)

    x_copies = [
        pltpu.make_async_copy(ax_hbm, ax_v, sem_x.at[0]),
        pltpu.make_async_copy(bx_hbm, bx_v, sem_x.at[1]),
    ]
    weights_unit(0)
    for priority, c in enumerate(x_copies):
        c.start(priority=priority)
    issue(weights_unit, 1, _UNITS - 1)
    issue(latent_unit, 0, _LAG)

    def build_expand(i, _):
        r0 = pl.multiple_of(i * 16, 16)
        row = lax.broadcasted_iota(jnp.int32, (16, 128 * _H), 0) + r0
        col = lax.broadcasted_iota(jnp.int32, (16, 128 * _H), 1)
        expand_s[pl.ds(r0, 16), :] = jnp.where(col // _H == row, 1.0, 0.0).astype(_BF16)

    _loop(128 // 16, build_expand)

    def keep_own_head(x):
        row = lax.broadcasted_iota(jnp.int32, (_B * _H, 128), 0)
        col = lax.broadcasted_iota(jnp.int32, (_B * _H, 128), 1)
        own = row % _H == col % _H
        tiles = [
            jnp.where(own, x[:, t : t + 128], 0.0).astype(_BF16)
            for t in range(0, x.shape[1], 128)
        ]
        return jnp.concatenate(tiles, axis=1)

    def per_head_proj(x, w_ref, j):
        lhs = keep_own_head(_dot(x, expand_s[...]))
        return _dot(lhs, w_ref[pl.ds(pl.multiple_of(j * 4096, 4096), 4096), :])

    for c in x_copies:
        c.wait()
    xa = ax_v[...].astype(_F32)
    xb = bx_v[...].astype(_F32)
    sub = lax.broadcasted_iota(jnp.int32, (8, _D), 0)
    for j in range(4):
        cols = slice(j * 128, (j + 1) * 128)
        for b in range(_B):
            xa_s[j, pl.ds(b * _H, _H), :] = jnp.broadcast_to(xa[b : b + 1, cols], (_H, 128))
        xb_s[j] = jnp.where(
            sub == 0,
            jnp.broadcast_to(xb[0:1, cols], (8, 128)),
            jnp.broadcast_to(xb[1:2, cols], (8, 128)),
        )

    _wait_whole(bwq_v, sem_w.at[0])
    _wait_whole(awq_v, sem_w.at[1])

    def q_step(j, carry):
        qa, qb = carry
        w = bwq_v[pl.ds(pl.multiple_of(j * 128, 128), 128), :]
        qb = qb + _dot(xb_s[j].astype(_BF16), w)
        qa = qa + per_head_proj(xa_s[j].astype(_BF16), awq_v, j)
        latent_unit(_LAG + j)
        return qa, qb

    qa, qb = _loop(
        4, q_step, (jnp.zeros((_B * _H, _D), _F32), jnp.zeros((8, _H * _D), _F32))
    )
    for h in range(_H):
        for b in range(_B):
            qb_s[pl.ds(b * _H + h, 1), :] = qb[b : b + 1, h * _D : (h + 1) * _D]
    qa = qa.astype(_BF16)

    _wait_whole(awuk_v, sem_w.at[2])
    _wait_whole(awuv_v, sem_w.at[3])

    kv_lag = _LAG * 4 // _G

    def absorb_step(j, _):
        w = awuk_v[pl.ds(pl.multiple_of(j * 4096, 4096), 4096), :]
        qa_s[j] = _nt_dot(keep_own_head(_nt_dot(qa, w)), expand_s[...])
        pl.when(j < 2)(lambda: latent_unit(_LAG + 4 + j))
        pl.when(j == 2)(lambda: kv_unit(0, 0))
        pl.when(j == 3)(lambda: kv_unit(0, 1))

    _loop(4, absorb_step)

    _wait_whole(ckv_v, sem_w.at[4])
    scale = _D ** -0.5
    kv_issued = kv_lag

    def latent_batch(b, _):
        heads = pl.ds(pl.multiple_of(b * _H, _H), _H)
        q = jnp.concatenate([qa_s[j, heads, :] for j in range(4)], axis=1).astype(_BF16)

        def block(j, carry):
            m, l, acc = carry
            c = ckv_v[pl.ds(pl.multiple_of(b * _S + j * 1024, 1024), 1024), :]
            s = _nt_dot(q, c)
            m_new = jnp.maximum(m, jnp.max(s, axis=1, keepdims=True))
            alpha = jnp.exp((m - m_new) * scale)
            p = jnp.exp((s - m_new) * scale)
            l = alpha * l + jnp.sum(p, axis=1, keepdims=True)
            acc = alpha * acc + _dot(p.astype(_BF16), c)
            kv_unit(kv_issued + b * 4 + j)
            return m_new, l, acc

        init = (
            jnp.full((_H, 1), -jnp.inf, _F32),
            jnp.zeros((_H, 1), _F32),
            jnp.zeros((_H, _M), _F32),
        )
        _, l, acc = _loop(4, block, init)
        cc = acc / l
        for j in range(4):
            cc_s[j, heads, :] = cc[:, j * 128 : (j + 1) * 128]

    _loop(_B, latent_batch)
    kv_issued += 8

    def value_step(j, ctx):
        ctx = ctx + per_head_proj(cc_s[j].astype(_BF16), awuv_v, j)
        if _G == 4:
            kv_unit(kv_issued + j)
        else:
            pl.when(j % 2 == 0)(lambda: kv_unit(kv_issued + j // 2))
        return ctx

    ctx_s[...] = _loop(4, value_step, jnp.zeros((_B * _H, _D), _F32))
    kv_issued += 16 // _G

    n_heads = _B * _H
    per_head = _UNITS // _G
    kv_steps = n_heads - kv_issued // per_head
    assert _UNITS + kv_lag <= kv_issued <= (_NSLOT - 1) * _UNITS
    out_slots = n_heads - kv_steps
    assert out_slots >= _UNITS

    def issue_out_weights(j):
        first = j * _UNITS // out_slots
        pl.when((j + 1) * _UNITS // out_slots > first)(lambda: out_weights_unit(first))

    def head_step(t, _):
        group, i = t // _G, t % _G
        slot = group % _NSLOT

        def issue_half(half):
            if _G == 4:
                pl.when(t < kv_steps)(lambda: kv_unit(kv_issued + 2 * t + half))
            else:
                pl.when(t < kv_steps)(lambda: kv_unit(kv_issued + t, half))
            if half == 0:
                pl.when(t >= kv_steps)(lambda: issue_out_weights(t - kv_steps))

        pl.when(i == 0)(lambda: _wait_whole(kv_v.at[slot], sem_kv.at[slot]))
        q = jnp.broadcast_to(qb_s[pl.ds(t, 1), :], (8, _D)).astype(_BF16)
        s = _nt_dot(q, kv_v[slot, 0, i])
        issue_half(0)
        m = jnp.max(s, axis=1, keepdims=True)
        p = jnp.exp((s - m) * scale)
        l = jnp.sum(p, axis=1, keepdims=True)
        o = _dot(p.astype(_BF16), kv_v[slot, 1, i])
        ob_s[pl.ds(t, 1), :] = (o / l)[0:1]
        issue_half(1)

    _loop(n_heads, head_step)

    def head_rows(ref, h):
        r0 = jnp.broadcast_to(ref[pl.ds(h, 1), :], (8, _D))
        r1 = jnp.broadcast_to(ref[pl.ds(_H + h, 1), :], (8, _D))
        return jnp.where(sub == 0, r0, r1).astype(_BF16)

    def out_step(piece, acc):
        _wait_whole(wo_v.at[piece], sem_o.at[piece])
        acc = list(acc)
        for which, src in enumerate((ctx_s, ob_s)):
            for q in range(4):
                lhs = head_rows(src, q * 8 + piece)
                acc[which] = acc[which] + _dot(lhs, wo_v[piece, which, q])
        return tuple(acc)

    acc = _loop(_UNITS, out_step, (jnp.zeros((8, _M), _F32),) * 2)
    out_ref[...] = jnp.concatenate(acc, axis=1)[0:_B].astype(out_ref.dtype)


@jax.jit
def pallas_concat_heads__compressed_kv_cla__gqa_block_cached__decode_kernel(
    A_x: jax.Array,
    A_c_kv: jax.Array,
    A_w_q: jax.Array,
    A_w_uk: jax.Array,
    A_w_uv: jax.Array,
    A_w_o: jax.Array,
    B_x: jax.Array,
    B_k_cache: jax.Array,
    B_v_cache: jax.Array,
    B_wq: jax.Array,
    B_wo: jax.Array,
):
    assert A_x.shape == B_x.shape == (_B, 1, _M)
    assert A_c_kv.shape == (_B, _S, _M)
    assert A_w_q.shape == A_w_uk.shape == A_w_uv.shape == (_M, _H, _D)
    assert B_k_cache.shape == B_v_cache.shape == (_B, _H, _S, _D)

    hbm = pl.BlockSpec(memory_space=pltpu.HBM)
    dma = pltpu.SemaphoreType.DMA
    out = pl.pallas_call(
        _kernel,
        in_specs=[hbm] * 11,
        out_specs=pl.BlockSpec(memory_space=pltpu.VMEM),
        out_shape=jax.ShapeDtypeStruct((_B, 2 * _M), A_x.dtype),
        scratch_shapes=[
            pltpu.VMEM((_B, _M), _BF16),
            pltpu.VMEM((_B, _M), _BF16),
            pltpu.VMEM((_M, _H * _D), _BF16),
            pltpu.VMEM((_M * _H, _D), _BF16),
            pltpu.VMEM((_M * _H, _D), _BF16),
            pltpu.VMEM((_M * _H, _D), _BF16),
            pltpu.VMEM((_B * _S, _M), _BF16),
            pltpu.VMEM((_UNITS, 2, 4, _D, _M), _BF16),
            pltpu.VMEM((_NSLOT, 2, _G, _S, _D), _BF16),
            pltpu.VMEM((128, 128 * _H), _BF16),
            pltpu.VMEM((4, _B * _H, 128), _F32),
            pltpu.VMEM((4, 8, 128), _F32),
            pltpu.VMEM((_B * _H, _D), _F32),
            pltpu.VMEM((_B * _H, _D), _F32),
            pltpu.VMEM((4, _B * _H, 128), _F32),
            pltpu.VMEM((4, _B * _H, 128), _F32),
            pltpu.VMEM((_B * _H, _D), _F32),
            dma((2,)),
            dma((5,)),
            dma((_NSLOT,)),
            dma((_UNITS,)),
        ],
        compiler_params=pltpu.CompilerParams(
            vmem_limit_bytes=100 * 2**20,
            disable_bounds_checks=True,
            disable_semaphore_checks=True,
        ),
    )(
        A_x.reshape(_B, _M),
        A_c_kv.reshape(_B * _S, _M),
        A_w_q.reshape(_M * _H, _D),
        A_w_uk.reshape(_M * _H, _D),
        A_w_uv.reshape(_M * _H, _D),
        A_w_o.reshape(_H * _D, _M),
        B_x.reshape(_B, _M),
        B_k_cache.reshape(_B * _H, _S, _D),
        B_v_cache.reshape(_B * _H, _S, _D),
        B_wq,
        B_wo,
    )
    return out.reshape(_B, 1, 2 * _M)
```

```python
import jax
import jax.numpy as jnp
from jax import lax
import jax.experimental.pallas as pl
import jax.experimental.pallas.tpu as pltpu

_BF16 = jnp.bfloat16
_F32 = jnp.float32

_B = 2
_H = 32
_D = 128
_M = 512
_S = 4096

_G = 8
_NSLOT = 3
_UNITS = 8
_KV_UNITS = 16
_BLK = 1024
_LAT = 512


def _chunks(*sizes):
    return tuple((sum(sizes[:i]), n) for i, n in enumerate(sizes))


_ROWS128 = _chunks(128, 64, 192, 64, 64)
_ROWS512 = _chunks(32, 16, 48, 16, 16)
_COLS4096 = _chunks(2048, 1024, 1024, 2048, 2048)


def _ds(start, size, align):
    return pl.ds(pl.multiple_of(start, align), size)


def _loop(n, body, init=None):
    return lax.fori_loop(0, n, body, init)


def _start_alternating(n, copies_of):
    def body(i, _):
        for j, (src, dst, sem) in enumerate(copies_of(i)):
            pltpu.make_async_copy(src, dst, sem).start(priority=j % 2)

    _loop(n, body)


def _wait_whole(buf, sem):
    pltpu.make_async_copy(buf, buf, sem).wait()


def _paced(step, steps, count, fn):
    assert count <= steps
    n = step * count // steps
    pl.when((step + 1) * count // steps > n)(lambda: fn(n))


def _nt_dot(a, b):
    return lax.dot_general(a, b, (((1,), (1,)), ((), ())), preferred_element_type=_F32)


def _dot(a, b):
    return jnp.dot(a, b, preferred_element_type=_F32)


def _kernel(
    ax_hbm, ckv_hbm, awq_hbm, awuk_hbm, awuv_hbm, awo_hbm,
    bx_hbm, k_hbm, v_hbm, bwq_hbm, bwo_hbm,
    out_ref,
    ax_v, bx_v, bwq_v, aw_v, ckv_v, wo_v, kv_v,
    expand_s, qb_s, ob_s, qa_s, proj_in_s, proj_out_s,
    sem_x, sem_w, sem_kv, sem_o,
):
    n_heads = _B * _H
    scale = _D ** -0.5

    def q_weights_unit(u):
        for (r, n), (c, m) in zip(_ROWS128, _COLS4096):

            def copies(q):
                tile = (_ds(q * 128 + u * 16 + c // 4096 * 8, 8, 8), pl.ds(c % 4096, m))
                rows = _ds(q * 4096 + u * 512 + r, n, 64)
                return [
                    (bwq_hbm.at[tile], bwq_v.at[tile], sem_w.at[0]),
                    (awq_hbm.at[rows], aw_v.at[0, rows], sem_w.at[1]),
                ]

            _start_alternating(4, copies)

    def up_weights_unit(u):
        for r, n in _ROWS128:

            def copies(q):
                rows = _ds(q * 4096 + u * 512 + r, n, 64)
                return [
                    (awuv_hbm.at[rows], aw_v.at[1, rows], sem_w.at[2]),
                    (awuk_hbm.at[rows], aw_v.at[2, rows], sem_w.at[2]),
                ]

            _start_alternating(4, copies)

    def latent_unit(u):
        for r, n in _ROWS512:

            def copies(q):
                rows = [_ds((2 * q + i) * 1024 + u * 128 + r, n, 16) for i in range(2)]
                return [(ckv_hbm.at[x], ckv_v.at[x], sem_w.at[3]) for x in rows]

            _start_alternating(4, copies)

    def kv_unit(u):
        group, k = u // _KV_UNITS, u % _KV_UNITS
        slot = group % _NSLOT

        def start(r, n):
            rows = _ds(r, n, 64)
            _start_alternating(_G, lambda i: [
                (src.at[group * _G + i, rows], kv_v.at[slot, which, i, rows], sem_kv.at[slot])
                for which, src in enumerate((k_hbm, v_hbm))
            ])

        start(k * 256 + 128, 64)
        pl.when(k < _KV_UNITS - 1)(lambda: start(k * 256 + 192, 192))

        @pl.when(k == _KV_UNITS - 1)
        def _():
            start(k * 256 + 192, 64)
            start(k * 0, 128)

    def out_weights_unit(u):
        def copies(q, r, n, sem):
            return [
                (
                    src.at[_ds(q * 1024 + u * 128 + r, n, 16)],
                    wo_v.at[u, which, q, pl.ds(r, n)],
                    sem,
                )
                for which, src in enumerate((awo_hbm, bwo_hbm))
            ]

        @pl.when(u < _UNITS - 1)
        def _():
            for r, n in _ROWS512:
                _start_alternating(4, lambda q: copies(q, r, n, sem_o.at[u]))

        @pl.when(u == _UNITS - 1)
        def _():
            _start_alternating(4, lambda q: [
                c for r, n in _ROWS512 for c in copies(q, r, n, sem_o.at[u + q])
            ])

    x_copies = [
        pltpu.make_async_copy(ax_hbm, ax_v, sem_x.at[0]),
        pltpu.make_async_copy(bx_hbm, bx_v, sem_x.at[1]),
    ]
    for priority, copy in enumerate(x_copies):
        copy.start(priority=priority)
    _loop(_UNITS, lambda u, _: q_weights_unit(u))
    _loop(2, lambda u, _: up_weights_unit(u))

    def build_expand(i, _):
        k, r0 = i // 8, i % 8 * 16
        row = lax.broadcasted_iota(jnp.int32, (16, _BLK), 0) + r0
        col = lax.broadcasted_iota(jnp.int32, (16, _BLK), 1) + k * _BLK
        hit = (col >= row * _H) & (col < (row + 1) * _H)
        expand_s[k, _ds(r0, 16, 16), :] = jnp.where(hit, 1.0, 0.0).astype(_BF16)

    per_block = 128 * _H // _BLK
    steps = 4 * per_block
    _loop(8 * per_block, build_expand)

    def keep_own_head(x):
        row = lax.broadcasted_iota(jnp.int32, (n_heads, 128), 0)
        col = lax.broadcasted_iota(jnp.int32, (n_heads, 128), 1)
        own = (row & (_H - 1)) == (col & (_H - 1))
        tiles = [
            jnp.where(own, x[:, t : t + 128], 0.0).astype(_BF16)
            for t in range(0, x.shape[1], 128)
        ]
        return jnp.concatenate(tiles, axis=1)

    def batch_rows(r0, r1):
        shape = (8, r0.shape[1])
        first = lax.broadcasted_iota(jnp.int32, shape, 0) == 0
        rows = jnp.where(first, jnp.broadcast_to(r0, shape), jnp.broadcast_to(r1, shape))
        return rows.astype(_BF16)

    for copy in x_copies:
        copy.wait()
    xa = ax_v[...].astype(_F32)
    for j in range(4):
        for b in range(_B):
            x = xa[b : b + 1, j * 128 : (j + 1) * 128]
            proj_in_s[j, pl.ds(b * _H, _H), :] = jnp.broadcast_to(x, (_H, 128))
    xb = bx_v[...].astype(_F32)
    xb = batch_rows(xb[0:1], xb[1:2])

    _wait_whole(bwq_v, sem_w.at[0])
    _wait_whole(aw_v.at[0], sem_w.at[1])

    def cached_q_step(i, _):
        q = _dot(xb, bwq_v[:, _ds(i * 2 * _D, 2 * _D, 2 * _D)])
        for h in range(2):
            for b in range(_B):
                qb_s[pl.ds(b * _H + 2 * i + h, 1), :] = q[b : b + 1, h * _D : (h + 1) * _D]
        _paced(i, _H // 2, 4, lambda n: up_weights_unit(2 + n))

    _loop(_H // 2, cached_q_step)

    def per_head_proj(stage):
        def step(i, acc):
            x = proj_in_s[i // per_block].astype(_BF16)
            lhs = keep_own_head(_dot(x, expand_s[i % per_block]))
            acc = acc + _dot(lhs, aw_v[stage, _ds(i * _BLK, _BLK, _BLK), :])

            def issue(n):
                pl.when((stage == 0) & (n < 2))(lambda: up_weights_unit(6 + n))
                pl.when((stage == 0) & (n >= 2))(lambda: latent_unit(n - 2))
                pl.when(stage == 1)(lambda: kv_unit(17 + n))

            _paced(i, steps, 7, issue)
            return acc

        proj_out_s[...] = _loop(steps, step, jnp.zeros((n_heads, _D), _F32))

    def absorb_keys():
        q = proj_out_s[...].astype(_BF16)
        qa_s[...] = jnp.zeros(qa_s.shape, _F32)

        def step(i, _):
            full = _nt_dot(q, aw_v[2, _ds(i * _BLK, _BLK, _BLK), :])
            qa_s[i // per_block] += _nt_dot(keep_own_head(full), expand_s[i % per_block])

            def issue(n):
                pl.when(n < 3)(lambda: latent_unit(5 + n))
                pl.when(n >= 3)(lambda: kv_unit(n - 3))

            _paced(i, steps, 7, issue)

        _loop(steps, step)

    def attend_latent(b, _):
        heads = _ds(b * _H, _H, _H)
        q = jnp.concatenate([qa_s[j, heads, :] for j in range(4)], axis=1).astype(_BF16)
        blocks = _S // _LAT

        def step(j, carry):
            m, l, acc = carry
            c = ckv_v[_ds(b * _S + j * _LAT, _LAT, _LAT), :]
            s = _nt_dot(q, c)
            m_new = jnp.maximum(m, jnp.max(s, axis=1, keepdims=True))
            alpha = jnp.exp((m - m_new) * scale)
            p = jnp.exp((s - m_new) * scale)
            l = alpha * l + jnp.sum(p, axis=1, keepdims=True)
            acc = alpha * acc + _dot(p.astype(_BF16), c)
            _paced(b * blocks + j, _B * blocks, 13, lambda n: kv_unit(4 + n))
            return m_new, l, acc

        init = (
            jnp.full((_H, 1), float(jnp.finfo(_F32).min), _F32),
            jnp.zeros((_H, 1), _F32),
            jnp.zeros((_H, _M), _F32),
        )
        _, l, acc = _loop(blocks, step, init)
        ctx = acc / l
        for j in range(4):
            proj_in_s[j, heads, :] = ctx[:, j * 128 : (j + 1) * 128]

    def latent_stage(stage, _):
        per_head_proj(stage)

        @pl.when(stage == 0)
        def _():
            _wait_whole(aw_v.at[pl.ds(1, 2)], sem_w.at[2])
            absorb_keys()
            _wait_whole(ckv_v, sem_w.at[3])
            _loop(_B, attend_latent)

    _loop(2, latent_stage)
    kv_issued = 24

    kv_steps = n_heads - kv_issued // 2
    out_slots = n_heads - kv_steps
    assert _KV_UNITS < kv_issued <= (_NSLOT - 1) * _KV_UNITS and out_slots >= _UNITS

    def head_step(t, _):
        group, i = t // _G, t % _G
        slot = group % _NSLOT
        pl.when(i == 0)(lambda: _wait_whole(kv_v.at[slot], sem_kv.at[slot]))
        q = jnp.broadcast_to(qb_s[pl.ds(t, 1), :], (8, _D)).astype(_BF16)
        s = _nt_dot(q, kv_v[slot, 0, i])
        pl.when(t < kv_steps)(lambda: kv_unit(kv_issued + 2 * t))

        pl.when(t >= kv_steps)(
            lambda: _paced(t - kv_steps, out_slots, _UNITS, out_weights_unit)
        )
        m = jnp.max(s, axis=1, keepdims=True)
        p = jnp.exp((s - m) * scale)
        l = jnp.sum(p, axis=1, keepdims=True)
        o = _dot(p.astype(_BF16), kv_v[slot, 1, i])
        ob_s[pl.ds(t, 1), :] = (o / l)[0:1]
        pl.when(t < kv_steps)(lambda: kv_unit(kv_issued + 2 * t + 1))

    _loop(n_heads, head_step)

    def project_out(u, q, acc):
        h = q * _UNITS + u
        return tuple(
            a + _dot(batch_rows(src[pl.ds(h, 1), :], src[pl.ds(_H + h, 1), :]), wo_v[u, which, q])
            for which, (a, src) in enumerate(zip(acc, (proj_out_s, ob_s)))
        )

    def out_step(u, acc):
        _wait_whole(wo_v.at[u], sem_o.at[u])
        for q in range(4):
            acc = project_out(u, q, acc)
        return acc

    def last_out_step(q, acc):
        _wait_whole(wo_v.at[_UNITS - 1, :, q], sem_o.at[_UNITS - 1 + q])
        return project_out(_UNITS - 1, q, acc)

    acc = _loop(_UNITS - 1, out_step, (jnp.zeros((8, _M), _F32),) * 2)
    acc = _loop(4, last_out_step, acc)
    out_ref[...] = jnp.concatenate(acc, axis=1)[0:_B].astype(out_ref.dtype)


@jax.jit
def pallas_concat_heads__compressed_kv_cla__gqa_block_cached__decode_kernel(
    A_x: jax.Array,
    A_c_kv: jax.Array,
    A_w_q: jax.Array,
    A_w_uk: jax.Array,
    A_w_uv: jax.Array,
    A_w_o: jax.Array,
    B_x: jax.Array,
    B_k_cache: jax.Array,
    B_v_cache: jax.Array,
    B_wq: jax.Array,
    B_wo: jax.Array,
):
    assert A_x.shape == B_x.shape == (_B, 1, _M)
    assert A_c_kv.shape == (_B, _S, _M)
    assert A_w_q.shape == A_w_uk.shape == A_w_uv.shape == (_M, _H, _D)
    assert B_k_cache.shape == B_v_cache.shape == (_B, _H, _S, _D)

    hbm = pl.BlockSpec(memory_space=pltpu.HBM)
    dma = pltpu.SemaphoreType.DMA
    out = pl.pallas_call(
        _kernel,
        in_specs=[hbm] * 11,
        out_specs=pl.BlockSpec(memory_space=pltpu.VMEM),
        out_shape=jax.ShapeDtypeStruct((_B, 2 * _M), A_x.dtype),
        scratch_shapes=[
            pltpu.VMEM((_B, _M), _BF16),
            pltpu.VMEM((_B, _M), _BF16),
            pltpu.VMEM((_M, _H * _D), _BF16),
            pltpu.VMEM((3, _M * _H, _D), _BF16),
            pltpu.VMEM((_B * _S, _M), _BF16),
            pltpu.VMEM((_UNITS, 2, 4, _D, _M), _BF16),
            pltpu.VMEM((_NSLOT, 2, _G, _S, _D), _BF16),
            pltpu.VMEM((128 * _H // _BLK, 128, _BLK), _BF16),
            pltpu.VMEM((_B * _H, _D), _F32),
            pltpu.VMEM((_B * _H, _D), _F32),
            pltpu.VMEM((4, _B * _H, 128), _F32),
            pltpu.VMEM((4, _B * _H, 128), _F32),
            pltpu.VMEM((_B * _H, _D), _F32),
            dma((2,)),
            dma((4,)),
            dma((_NSLOT,)),
            dma((_UNITS + 3,)),
        ],
        compiler_params=pltpu.CompilerParams(
            vmem_limit_bytes=100 * 2**20,
            disable_bounds_checks=True,
            disable_semaphore_checks=True,
        ),
    )(
        A_x.reshape(_B, _M),
        A_c_kv.reshape(_B * _S, _M),
        A_w_q.reshape(_M * _H, _D),
        A_w_uk.reshape(_M * _H, _D),
        A_w_uv.reshape(_M * _H, _D),
        A_w_o.reshape(_H * _D, _M),
        B_x.reshape(_B, _M),
        B_k_cache.reshape(_B * _H, _S, _D),
        B_v_cache.reshape(_B * _H, _S, _D),
        B_wq,
        B_wo,
    )
    return out.reshape(_B, 1, 2 * _M)
```

```python
import jax
import jax.numpy as jnp
from jax import lax
import jax.experimental.pallas as pl
import jax.experimental.pallas.tpu as pltpu

_BF16 = jnp.bfloat16
_F32 = jnp.float32

_B = 2
_H = 32
_D = 128
_M = 512
_S = 4096

_G = 8
_NSLOT = 3
_UNITS = 8
_KV_UNITS = 16
_BLK = 1024
_LAT = 512


def _chunks(*sizes):
    return tuple((sum(sizes[:i]), n) for i, n in enumerate(sizes))


_ROWS128 = _chunks(128, 64, 192, 64, 64)
_ROWS512 = _chunks(32, 16, 48, 16, 16)
_COLS4096 = _chunks(2048, 1024, 1024, 2048, 2048)


def _ds(start, size, align):
    return pl.ds(pl.multiple_of(start, align), size)


def _loop(n, body, init=None):
    return lax.fori_loop(0, n, body, init)


def _start_alternating(n, copies_of):
    def body(i, _):
        for j, (src, dst, sem) in enumerate(copies_of(i)):
            pltpu.make_async_copy(src, dst, sem).start(priority=j % 2)

    _loop(n, body)


def _wait_whole(buf, sem):
    pltpu.make_async_copy(buf, buf, sem).wait()


def _paced(step, steps, count, fn):
    assert count <= steps
    n = step * count // steps
    pl.when((step + 1) * count // steps > n)(lambda: fn(n))


def _nt_dot(a, b):
    return lax.dot_general(a, b, (((1,), (1,)), ((), ())), preferred_element_type=_F32)


def _dot(a, b):
    return jnp.dot(a, b, preferred_element_type=_F32)


def _kernel(
    ax_hbm, ckv_hbm, awq_hbm, awuk_hbm, awuv_hbm, awo_hbm,
    bx_hbm, k_hbm, v_hbm, bwq_hbm, bwo_hbm,
    out_ref,
    ax_v, bx_v, bwq_v, aw_v, ckv_v, wo_v, kv_v,
    expand_s, qb_s, ob_s, qa_s, proj_in_s, proj_out_s,
    sem_x, sem_w, sem_kv, sem_o,
):
    n_heads = _B * _H
    scale = _D ** -0.5

    def q_weights_unit(u):
        for (r, n), (c, m) in zip(_ROWS128, _COLS4096):

            def copies(q):
                tile = (_ds(q * 128 + u * 16 + c // 4096 * 8, 8, 8), pl.ds(c % 4096, m))
                rows = _ds(q * 4096 + u * 512 + r, n, 64)
                return [
                    (bwq_hbm.at[tile], bwq_v.at[tile], sem_w.at[0]),
                    (awq_hbm.at[rows], aw_v.at[0, rows], sem_w.at[1]),
                ]

            _start_alternating(4, copies)

    def up_weights_unit(u):
        for r, n in _ROWS128:

            def copies(q):
                rows = _ds(q * 4096 + u * 512 + r, n, 64)
                return [
                    (awuv_hbm.at[rows], aw_v.at[1, rows], sem_w.at[2]),
                    (awuk_hbm.at[rows], aw_v.at[2, rows], sem_w.at[2]),
                ]

            _start_alternating(4, copies)

    def latent_unit(u):
        for r, n in _ROWS512:

            def copies(q):
                rows = [_ds((2 * q + i) * 1024 + u * 128 + r, n, 16) for i in range(2)]
                return [(ckv_hbm.at[x], ckv_v.at[x], sem_w.at[3]) for x in rows]

            _start_alternating(4, copies)

    def kv_unit(u):
        group, k = u // _KV_UNITS, u % _KV_UNITS
        slot = group % _NSLOT

        def start(r, n):
            rows = _ds(r, n, 64)
            _start_alternating(_G, lambda i: [
                (src.at[group * _G + i, rows], kv_v.at[slot, which, i, rows], sem_kv.at[slot])
                for which, src in enumerate((k_hbm, v_hbm))
            ])

        start(k * 256 + 128, 64)
        pl.when(k < _KV_UNITS - 1)(lambda: start(k * 256 + 192, 192))

        @pl.when(k == _KV_UNITS - 1)
        def _():
            start(k * 256 + 192, 64)
            start(k * 0, 128)

    def out_weights_unit(u):
        def copies(q, r, n, sem):
            return [
                (
                    src.at[_ds(q * 1024 + u * 128 + r, n, 16)],
                    wo_v.at[u, which, q, pl.ds(r, n)],
                    sem,
                )
                for which, src in enumerate((awo_hbm, bwo_hbm))
            ]

        @pl.when(u < _UNITS - 1)
        def _():
            for r, n in _ROWS512:
                _start_alternating(4, lambda q: copies(q, r, n, sem_o.at[u]))

        @pl.when(u == _UNITS - 1)
        def _():
            _start_alternating(4, lambda q: [
                c for r, n in _ROWS512 for c in copies(q, r, n, sem_o.at[u + q])
            ])

    x_copies = [
        pltpu.make_async_copy(ax_hbm, ax_v, sem_x.at[0]),
        pltpu.make_async_copy(bx_hbm, bx_v, sem_x.at[1]),
    ]
    for priority, copy in enumerate(x_copies):
        copy.start(priority=priority)
    _loop(_UNITS, lambda u, _: q_weights_unit(u))
    _loop(2, lambda u, _: up_weights_unit(u))

    def build_expand(i, _):
        k, r0 = i // 8, i % 8 * 16
        row = lax.broadcasted_iota(jnp.int32, (16, _BLK), 0) + r0
        col = lax.broadcasted_iota(jnp.int32, (16, _BLK), 1) + k * _BLK
        hit = (col >= row * _H) & (col < (row + 1) * _H)
        expand_s[k, _ds(r0, 16, 16), :] = jnp.where(hit, 1.0, 0.0).astype(_BF16)

    per_block = 128 * _H // _BLK
    steps = 4 * per_block
    _loop(8 * per_block, build_expand)

    def keep_own_head(x):
        row = lax.broadcasted_iota(jnp.int32, (n_heads, 128), 0)
        col = lax.broadcasted_iota(jnp.int32, (n_heads, 128), 1)
        own = (row & (_H - 1)) == (col & (_H - 1))
        tiles = [
            jnp.where(own, x[:, t : t + 128], 0.0).astype(_BF16)
            for t in range(0, x.shape[1], 128)
        ]
        return jnp.concatenate(tiles, axis=1)

    def batch_rows(r0, r1):
        shape = (8, r0.shape[1])
        first = lax.broadcasted_iota(jnp.int32, shape, 0) == 0
        rows = jnp.where(first, jnp.broadcast_to(r0, shape), jnp.broadcast_to(r1, shape))
        return rows.astype(_BF16)

    for copy in x_copies:
        copy.wait()
    xa = ax_v[...].astype(_F32)
    for j in range(4):
        for b in range(_B):
            x = xa[b : b + 1, j * 128 : (j + 1) * 128]
            proj_in_s[j, pl.ds(b * _H, _H), :] = jnp.broadcast_to(x, (_H, 128))
    xb = bx_v[...].astype(_F32)
    xb = batch_rows(xb[0:1], xb[1:2])

    _wait_whole(bwq_v, sem_w.at[0])
    _wait_whole(aw_v.at[0], sem_w.at[1])

    def cached_q_step(i, _):
        q = _dot(xb, bwq_v[:, _ds(i * 2 * _D, 2 * _D, 2 * _D)])
        for h in range(2):
            for b in range(_B):
                qb_s[pl.ds(b * _H + 2 * i + h, 1), :] = q[b : b + 1, h * _D : (h + 1) * _D]
        _paced(i, _H // 2, 4, lambda n: up_weights_unit(2 + n))

    _loop(_H // 2, cached_q_step)

    def per_head_proj(stage):
        def step(i, acc):
            x = proj_in_s[i // per_block].astype(_BF16)
            lhs = keep_own_head(_dot(x, expand_s[i % per_block]))
            acc = acc + _dot(lhs, aw_v[stage, _ds(i * _BLK, _BLK, _BLK), :])

            def issue(n):
                pl.when((stage == 0) & (n < 2))(lambda: up_weights_unit(6 + n))
                pl.when((stage == 0) & (n >= 2))(lambda: latent_unit(n - 2))
                pl.when(stage == 1)(lambda: kv_unit(17 + n))

            _paced(i, steps, 7, issue)
            return acc

        proj_out_s[...] = _loop(steps, step, jnp.zeros((n_heads, _D), _F32))

    def absorb_keys():
        q = proj_out_s[...].astype(_BF16)
        qa_s[...] = jnp.zeros(qa_s.shape, _F32)

        def step(i, _):
            full = _nt_dot(q, aw_v[2, _ds(i * _BLK, _BLK, _BLK), :])
            qa_s[i // per_block] += _nt_dot(keep_own_head(full), expand_s[i % per_block])

            def issue(n):
                pl.when(n < 3)(lambda: latent_unit(5 + n))
                pl.when(n >= 3)(lambda: kv_unit(n - 3))

            _paced(i, steps, 7, issue)

        _loop(steps, step)

    def attend_latent(b, _):
        heads = _ds(b * _H, _H, _H)
        q = jnp.concatenate([qa_s[j, heads, :] for j in range(4)], axis=1).astype(_BF16)
        blocks = _S // _LAT

        def step(j, carry):
            m, l, acc = carry
            c = ckv_v[_ds(b * _S + j * _LAT, _LAT, _LAT), :]
            s = _nt_dot(q, c)
            m_new = jnp.maximum(m, jnp.max(s, axis=1, keepdims=True))
            alpha = jnp.exp((m - m_new) * scale)
            p = jnp.exp((s - m_new) * scale)
            l = alpha * l + jnp.sum(p, axis=1, keepdims=True)
            acc = alpha * acc + _dot(p.astype(_BF16), c)
            _paced(b * blocks + j, _B * blocks, 13, lambda n: kv_unit(4 + n))
            return m_new, l, acc

        init = (
            jnp.full((_H, 1), float(jnp.finfo(_F32).min), _F32),
            jnp.zeros((_H, 1), _F32),
            jnp.zeros((_H, _M), _F32),
        )
        _, l, acc = _loop(blocks, step, init)
        ctx = acc / l
        for j in range(4):
            proj_in_s[j, heads, :] = ctx[:, j * 128 : (j + 1) * 128]

    def latent_stage(stage, _):
        per_head_proj(stage)

        @pl.when(stage == 0)
        def _():
            _wait_whole(aw_v.at[pl.ds(1, 2)], sem_w.at[2])
            absorb_keys()
            _wait_whole(ckv_v, sem_w.at[3])
            _loop(_B, attend_latent)

    _loop(2, latent_stage)
    kv_issued = 24

    kv_steps = n_heads - kv_issued // 2
    out_slots = n_heads - kv_steps
    assert _KV_UNITS < kv_issued <= (_NSLOT - 1) * _KV_UNITS and out_slots >= _UNITS

    def head_step(t, _):
        group, i = t // _G, t % _G
        slot = group % _NSLOT
        pl.when(i == 0)(lambda: _wait_whole(kv_v.at[slot], sem_kv.at[slot]))
        q = jnp.broadcast_to(qb_s[pl.ds(t, 1), :], (8, _D)).astype(_BF16)
        s = _nt_dot(q, kv_v[slot, 0, i])
        pl.when(t < kv_steps)(lambda: kv_unit(kv_issued + 2 * t))
        pl.when(t >= kv_steps)(
            lambda: _paced(t - kv_steps, out_slots, _UNITS, out_weights_unit)
        )
        m = jnp.max(s, axis=1, keepdims=True)
        p = jnp.exp((s - m) * scale)
        l = jnp.sum(p, axis=1, keepdims=True)
        o = _dot(p.astype(_BF16), kv_v[slot, 1, i])
        ob_s[pl.ds(t, 1), :] = (o / l)[0:1]
        pl.when(t < kv_steps)(lambda: kv_unit(kv_issued + 2 * t + 1))

    _loop(n_heads, head_step)

    def project_out(u, q, acc):
        h = q * _UNITS + u
        heads = [
            batch_rows(src[pl.ds(h, 1), :], src[pl.ds(_H + h, 1), :])
            for src in (proj_out_s, ob_s)
        ]
        return tuple(acc[i] + _dot(heads[i], wo_v[u, i, q]) for i in range(2))

    def out_step(u, acc):
        _wait_whole(wo_v.at[u], sem_o.at[u])
        for q in range(4):
            acc = project_out(u, q, acc)
        return acc

    def last_out_step(q, acc):
        _wait_whole(wo_v.at[_UNITS - 1, :, q], sem_o.at[_UNITS - 1 + q])
        return project_out(_UNITS - 1, q, acc)

    acc = _loop(_UNITS - 1, out_step, (jnp.zeros((8, _M), _F32),) * 2)
    acc = _loop(4, last_out_step, acc)
    out_ref[...] = jnp.concatenate(acc, axis=1)[0:_B].astype(out_ref.dtype)


@jax.jit
def pallas_concat_heads__compressed_kv_cla__gqa_block_cached__decode_kernel(
    A_x: jax.Array,
    A_c_kv: jax.Array,
    A_w_q: jax.Array,
    A_w_uk: jax.Array,
    A_w_uv: jax.Array,
    A_w_o: jax.Array,
    B_x: jax.Array,
    B_k_cache: jax.Array,
    B_v_cache: jax.Array,
    B_wq: jax.Array,
    B_wo: jax.Array,
):
    assert A_x.shape == B_x.shape == (_B, 1, _M)
    assert A_c_kv.shape == (_B, _S, _M)
    assert A_w_q.shape == A_w_uk.shape == A_w_uv.shape == (_M, _H, _D)
    assert B_k_cache.shape == B_v_cache.shape == (_B, _H, _S, _D)

    hbm = pl.BlockSpec(memory_space=pltpu.HBM)
    dma = pltpu.SemaphoreType.DMA
    out = pl.pallas_call(
        _kernel,
        in_specs=[hbm] * 11,
        out_specs=pl.BlockSpec(memory_space=pltpu.VMEM),
        out_shape=jax.ShapeDtypeStruct((_B, 2 * _M), A_x.dtype),
        scratch_shapes=[
            pltpu.VMEM((_B, _M), _BF16),
            pltpu.VMEM((_B, _M), _BF16),
            pltpu.VMEM((_M, _H * _D), _BF16),
            pltpu.VMEM((3, _M * _H, _D), _BF16),
            pltpu.VMEM((_B * _S, _M), _BF16),
            pltpu.VMEM((_UNITS, 2, 4, _D, _M), _BF16),
            pltpu.VMEM((_NSLOT, 2, _G, _S, _D), _BF16),
            pltpu.VMEM((128 * _H // _BLK, 128, _BLK), _BF16),
            pltpu.VMEM((_B * _H, _D), _F32),
            pltpu.VMEM((_B * _H, _D), _F32),
            pltpu.VMEM((4, _B * _H, 128), _F32),
            pltpu.VMEM((4, _B * _H, 128), _F32),
            pltpu.VMEM((_B * _H, _D), _F32),
            dma((2,)),
            dma((4,)),
            dma((_NSLOT,)),
            dma((_UNITS + 3,)),
        ],
        compiler_params=pltpu.CompilerParams(
            vmem_limit_bytes=100 * 2**20,
            disable_bounds_checks=True,
            disable_semaphore_checks=True,
        ),
    )(
        A_x.reshape(_B, _M),
        A_c_kv.reshape(_B * _S, _M),
        A_w_q.reshape(_M * _H, _D),
        A_w_uk.reshape(_M * _H, _D),
        A_w_uv.reshape(_M * _H, _D),
        A_w_o.reshape(_H * _D, _M),
        B_x.reshape(_B, _M),
        B_k_cache.reshape(_B * _H, _S, _D),
        B_v_cache.reshape(_B * _H, _S, _D),
        B_wq,
        B_wo,
    )
    return out.reshape(_B, 1, 2 * _M)
```
